```python
import os as _os
_os.environ.setdefault("JAX_PLATFORMS", "cpu")
import jax
import jax.numpy as jnp

def _softmax(x, axis=-1):
    return jax.nn.softmax(x, axis=axis)
def _gelu(x):
    return jax.nn.gelu(x, approximate=True)
def _silu(x):
    return jax.nn.silu(x)
def _sigmoid(x):
    return jax.nn.sigmoid(x)
def _layernorm(x, axis=-1, eps=1e-5):
    m = jnp.mean(x, axis=axis, keepdims=True)
    v = jnp.var(x, axis=axis, keepdims=True)
    return (x - m) / jnp.sqrt(v + eps)
def _scatter_add(tgt, idx, src, axis=0):
    return tgt.at[idx].add(src)
def _segment_sum(src, seg, n):
    return jax.ops.segment_sum(src, seg, n)
class _Rng:
    def __init__(self, key):
        self._k = key
    def _next(self):
        self._k, sub = jax.random.split(self._k)
        return sub
    def normal(self, shape):
        return jax.random.normal(self._next(), shape, dtype=jnp.bfloat16)
    def randint(self, lo, hi, shape):
        return jax.random.randint(self._next(), shape, lo, hi, dtype=jnp.int32)
    def uniform(self, shape, lo=0.0, hi=1.0):
        return jax.random.uniform(self._next(), shape, jnp.bfloat16, lo, hi)
    def permutation(self, n):
        return jax.random.permutation(self._next(), n)


kernel_name = 'standalone__mha_block_cached__near_ridge'

def setup_inputs():
    _rng = _Rng(jax.random.key(int.from_bytes(__import__("os").urandom(4), "little")))
    _w = (lambda a: (lambda t: t.astype(jnp.bfloat16) if jnp.issubdtype(t.dtype, jnp.floating) else t)(jnp.asarray(a)))
    B, Sq, D = 8, 96, 576
    H, Sk, Dh = 32, 96, 128
    return {
        "x": _w((lambda *s: _rng.normal(s) * 0.8)(B, Sq, D)),
        "k_cache": _w((lambda *s: _rng.normal(s) * 0.8)(B, H, Sk, Dh)),
        "v_cache": _w((lambda *s: _rng.normal(s) * 0.05)(B, H, Sk, Dh)),
        "wq": _w((lambda *s: _rng.normal(s) * 0.8)(D, H * Dh) * (D ** -0.5)),
        "wo": _w((lambda *s: _rng.normal(s) * 0.05)(H * Dh, D) * ((H * Dh) ** -0.5)),
    }

def reference(x, k_cache, v_cache, wq, wo):
    B, Sq, D = x.shape
    H, Dh = 32, 128
    q = (lambda x, *d: x.transpose(*d))((x @ wq).reshape(B, Sq, H, Dh), 0, 2, 1, 3)
    scores = jnp.einsum("bhqd,bhkd->bhqk", q, k_cache) * (Dh ** -0.5)
    p = _softmax(scores, axis=-1)
    o = jnp.einsum("bhqk,bhkd->bhqd", p, v_cache)
    return (lambda x, *d: x.transpose(*d))(o, 0, 2, 1, 3).reshape(B, Sq, H * Dh) @ wo
```

```python
import jax
import jax.numpy as jnp
import numpy as np
from jax.experimental import pallas as pl
from jax.experimental.pallas import tpu as pltpu

NT = (((1,), (1,)), ((), ()))
f32, bf16 = jnp.float32, jnp.bfloat16

def merge(*lists):
    items = []
    for li, l in enumerate(lists):
        n = len(l)
        for i, t in enumerate(l):
            items.append(((i + 0.5) / n, li, i, t))
    items.sort(key=lambda z: z[:3])
    return [t for *_, t in items]

def make(G=4, AR=128, LAG=4, UN=1):
    @jax.jit
    def pallas_standalone__mha_block_cached__near_ridge_kernel(x, k_cache, v_cache, wq, wo):
        B, Sq, D = x.shape
        _, H, Sk, Dh = k_cache.shape
        M = B * Sq
        c = float(Dh ** -0.5 * np.log2(np.e))
        NG = H // G
        GD = G * Dh
        TT = M // 128

        def kern(x_hbm, wq_hbm, k_hbm, v_hbm, wot_hbm, o_hbm,
                 x_v, wq_v, k_v, v_v, wot_v, acc, q_s, o_s, out_v, sems, xsem, osem):
            def cp(kind, g):
                cols = pl.ds(g * GD if isinstance(g, int) else pl.multiple_of(g * GD, GD), GD); hs = pl.ds(g * G, G)
                src, dst = [(wq_hbm.at[:, cols], wq_v), (k_hbm.at[:, hs], k_v),
                            (v_hbm.at[:, hs], v_v), (wot_hbm.at[:, cols], wot_v)][kind]
                return pltpu.make_async_copy(src, dst.at[g], sems.at[kind, g])
            xc = pltpu.make_async_copy(x_hbm, x_v, xsem)
            xc.start(); cp(0, 0).start()
            xc.wait()
            cp(1, 0).start(); cp(0, 1).start()
            cp(0, 0).wait()
            cp(2, 0).start(); cp(1, 1).start()

            def A(g, r):
                def f():
                    rows = slice(r * AR, (r + 1) * AR)
                    q_s[g, rows, :] = jnp.dot(x_v[rows, :], wq_v[g], preferred_element_type=f32).astype(bf16)
                return f
            st = {}
            def S(g, b, h):
                def f():
                    q = q_s[g, b * Sq:(b + 1) * Sq, h * Dh:(h + 1) * Dh]
                    s = jax.lax.dot_general(q, k_v[g, b, h], NT, preferred_element_type=f32)
                    m = jnp.max(s, axis=-1, keepdims=True)
                    p = jnp.exp2((s - m) * c)
                    l = jnp.sum(p, axis=-1, keepdims=True)
                    r = pl.reciprocal(l, approx=True)
                    r = r * (2.0 - l * r)
                    st[b, h] = (p.astype(bf16), r)
                return f
            def PV(g, b, h):
                def f():
                    p, r = st.pop((b, h))
                    o = jnp.dot(p, v_v[g, b, h], preferred_element_type=f32)
                    o_s[g, b * Sq:(b + 1) * Sq, h * Dh:(h + 1) * Dh] = (o * r).astype(bf16)
                return f
            def E(g, j, first, last):
                def f():
                    t = slice(j * 128, (j + 1) * 128)
                    res = jax.lax.dot_general(wot_v[g], o_s[g, t, :], NT, preferred_element_type=f32)
                    if not first:
                        res = res + acc[:, t]
                    if not last:
                        acc[:, t] = res
                    else:
                        out_v[t, :] = res.T.astype(bf16)
                        pltpu.make_async_copy(out_v.at[t, :], o_hbm.at[t, :], osem.at[j]).start()
                return f
            def attn(g):
                u = [(b, h) for b in range(B) for h in range(G)]
                l = []
                for i in range(len(u) + LAG):
                    if i < len(u): l.append(S(g, *u[i]))
                    if i >= LAG: l.append(PV(g, *u[i - LAG]))
                return l
            def stage(t, ts):
                if ts >= 0:
                    if ts + 2 < NG: cp(0, t + 2).start(); cp(1, t + 2).start()
                    if ts + 1 < NG: cp(2, t + 1).start()
                    if ts < NG: cp(3, t).start()
                    if ts + 1 < NG: cp(0, t + 1).wait()
                    if ts < NG: cp(1, t).wait(); cp(2, t).wait()
                    if ts >= 1: cp(3, t - 1).wait()
                ls = []
                if 0 <= ts + 1 < NG: ls.append([A(t + 1, r) for r in range(M // AR)])
                if 0 <= ts < NG: ls.append(attn(t))
                if 0 <= ts - 1 < NG: ls.append([E(t - 1, j, ts == 1, ts == NG) for j in range(TT)])
                for f in merge(*ls): f()
            lo, hi = 2, NG - 2
            for t in range(-1, lo): stage(t, t)
            def body(i, cc):
                for u in range(UN):
                    stage(lo + i * UN + u, lo)
                return cc
            assert (hi - lo) % UN == 0
            jax.lax.fori_loop(0, (hi - lo) // UN, body, 0)
            for t in range(hi, NG + 1): stage(t, t)
            for j in range(TT):
                t = slice(j * 128, (j + 1) * 128)
                pltpu.make_async_copy(out_v.at[t, :], o_hbm.at[t, :], osem.at[j]).wait()

        hbm = pl.BlockSpec(memory_space=pltpu.HBM)
        out = pl.pallas_call(
            kern,
            in_specs=[hbm] * 5,
            out_specs=hbm,
            out_shape=jax.ShapeDtypeStruct((M, D), x.dtype),
            scratch_shapes=[pltpu.VMEM((M, D), bf16),
                            pltpu.VMEM((NG, D, GD), bf16),
                            pltpu.VMEM((NG, B, G, Sk, Dh), bf16),
                            pltpu.VMEM((NG, B, G, Sk, Dh), bf16),
                            pltpu.VMEM((NG, D, GD), bf16),
                            pltpu.VMEM((D, M), f32),
                            pltpu.VMEM((NG, M, GD), bf16),
                            pltpu.VMEM((NG, M, GD), bf16),
                            pltpu.VMEM((M, D), bf16),
                            pltpu.SemaphoreType.DMA((4, NG)),
                            pltpu.SemaphoreType.DMA(()),
                            pltpu.SemaphoreType.DMA((TT,))],
            compiler_params=pltpu.CompilerParams(vmem_limit_bytes=100 * 1024 * 1024),
        )(x.reshape(M, D), wq, k_cache, v_cache, wo.T)
        return out.reshape(B, Sq, D)
    return pallas_standalone__mha_block_cached__near_ridge_kernel

pallas_standalone__mha_block_cached__near_ridge_kernel = make()
```
